```python
import os as _os
_os.environ.setdefault("JAX_PLATFORMS", "cpu")
import jax
import jax.numpy as jnp

def _softmax(x, axis=-1):
    return jax.nn.softmax(x, axis=axis)
def _gelu(x):
    return jax.nn.gelu(x, approximate=True)
def _silu(x):
    return jax.nn.silu(x)
def _sigmoid(x):
    return jax.nn.sigmoid(x)
def _layernorm(x, axis=-1, eps=1e-5):
    m = jnp.mean(x, axis=axis, keepdims=True)
    v = jnp.var(x, axis=axis, keepdims=True)
    return (x - m) / jnp.sqrt(v + eps)
def _scatter_add(tgt, idx, src, axis=0):
    return tgt.at[idx].add(src)
def _segment_sum(src, seg, n):
    return jax.ops.segment_sum(src, seg, n)
class _Rng:
    def __init__(self, key):
        self._k = key
    def _next(self):
        self._k, sub = jax.random.split(self._k)
        return sub
    def normal(self, shape):
        return jax.random.normal(self._next(), shape, dtype=jnp.bfloat16)
    def randint(self, lo, hi, shape):
        return jax.random.randint(self._next(), shape, lo, hi, dtype=jnp.int32)
    def uniform(self, shape, lo=0.0, hi=1.0):
        return jax.random.uniform(self._next(), shape, jnp.bfloat16, lo, hi)
    def permutation(self, n):
        return jax.random.permutation(self._next(), n)


kernel_name = 'sequential_preLN__sliding_block__swiglu_ffn__prompt'

def setup_inputs():
    _rng = _Rng(jax.random.key(int.from_bytes(__import__("os").urandom(4), "little")))
    _w = (lambda a: (lambda t: t.astype(jnp.bfloat16) if jnp.issubdtype(t.dtype, jnp.floating) else t)(jnp.asarray(a)))
    def _A_setup():
        B, S, D = 1, 2048, 512
        return {
            "x": _w((lambda *s: _rng.normal(s) * 0.05)(B, S, D)),
            "wqkv": _w((lambda *s: _rng.normal(s) * 0.05)(D, 3 * D)),
            "wo": _w((lambda *s: _rng.normal(s) * 0.05)(D, D)),
        }
    _A_in = _A_setup()

    def _B_setup():
        B, S, D, F = 1, 2048, 512, 1792
        return {
            "x": _w((lambda *s: _rng.normal(s) * 0.05)(B, S, D)),
            "w_gate": _w((lambda *s: _rng.normal(s) * 0.05)(D, F)),
            "w_up": _w((lambda *s: _rng.normal(s) * 0.05)(D, F)),
            "w_down": _w((lambda *s: _rng.normal(s) * 0.05)(F, D)),
        }
    _B_in = _B_setup()

    return {
        "A_x": _A_in["x"],
        "A_wqkv": _A_in["wqkv"],
        "A_wo": _A_in["wo"],
        "B_x": _B_in["x"],
        "B_w_gate": _B_in["w_gate"],
        "B_w_up": _B_in["w_up"],
        "B_w_down": _B_in["w_down"],
    }

def reference(A_x, A_wqkv, A_wo, B_x, B_w_gate, B_w_up, B_w_down):
    def _A_ref(x, wqkv, wo):
        B, S, D = x.shape
        H = 32; Dh = D // H; W = 256
        qkv = (lambda x, *d: x.transpose(*d))((x @ wqkv).reshape(B, S, 3, H, Dh), 2, 0, 3, 1, 4)
        q, k, v = qkv[0], qkv[1], qkv[2]
        scores = jnp.einsum("bhqd,bhkd->bhqk", q, k) * (Dh ** -0.5)
        idx = jnp.arange(S)
        mask = (idx[:, None] - idx[None, :] >= 0) & (idx[:, None] - idx[None, :] < W)
        scores = jnp.where(mask[None, None], scores, -1e9)
        p = _softmax(scores, axis=-1)
        o = jnp.einsum("bhqk,bhkd->bhqd", p, v)
        return (lambda x, *d: x.transpose(*d))(o, 0, 2, 1, 3).reshape(B, S, D) @ wo

    def _B_ref(x, w_gate, w_up, w_down):
        g = _silu(x @ w_gate)
        u = x @ w_up
        return (g * u) @ w_down

    x = A_x
    h = x + _A_ref(_layernorm(x, axis=-1), A_wqkv, A_wo)
    h2 = h + _B_ref(_layernorm(h, axis=-1), B_w_gate, B_w_up, B_w_down)
    return h2
```

```python
import functools
import jax
import jax.numpy as jnp
import numpy as np
from jax import lax
from jax.experimental import pallas as pl
from jax.experimental.pallas import tpu as pltpu

S, D, H, DH, W, F = 2048, 512, 32, 16, 256, 1792
TM = 256
NB = S // TM
EPS = 1e-5
SROWS = 4 * W + 32
QSCALE = float(DH ** -0.5 * np.log2(np.e))
NEG = -1e30
NT = (((1,), (1,)), ((), ()))
f32, bf16, i32 = jnp.float32, jnp.bfloat16, jnp.int32


def _ln(x):
    m = jnp.mean(x, axis=-1, keepdims=True)
    c = x - m
    v = jnp.mean(c * c, axis=-1, keepdims=True)
    return c * lax.rsqrt(v + EPS)


def _sel(bit, x, y):
    ln = lax.broadcasted_iota(i32, x.shape, 1)
    return jnp.where((ln & bit) == 0, x, y)


def _lo_valid():
    return lax.broadcasted_iota(i32, (16, 128), 0) > (lax.broadcasted_iota(i32, (16, 128), 1) & 15)


def _butterfly(xs):
    for bit, d in ((32, 1), (64, 2)):
        ys = []
        for u in range(4):
            x, y = xs[u], xs[u ^ d]
            if x is None and y is None:
                ys.append(None)
            else:
                ys.append(_sel(bit, jnp.zeros_like(y) if x is None else x, jnp.zeros_like(x) if y is None else y))
        xs = ys
    return xs


class _Attn:
    def __init__(self, a, qload, kload, vload, store, s_ref):
        self.a, self.qload, self.kload, self.vload, self.store, self.s_ref = a, qload, kload, vload, store, s_ref
        self.have, self.m, self.l = [None] * 4, [None] * 4, [None] * 4
        self.p = {}

    def scores(self):
        lane = lax.broadcasted_iota(i32, (8, 128), 1)
        for u in range(4):
            qu = self.qload(u)
            qbd = jnp.concatenate(
                [jnp.where((lane >> 4) == 4 * (s & 1) + ((s >> 1) ^ u), qu, 0) for s in range(8)], axis=0)
            back = min(W, self.a + 16 * u)
            st = lax.dot_general(self.kload(self.a + 16 * u - back, back + 16), pltpu.bitcast(qbd, bf16), NT,
                                 preferred_element_type=f32)
            nb = back // 16
            ch = {(u - nb + j) % 16: st[16 * j:16 * j + 16] for j in range(1 if back == W else 0, nb)}
            ch[u] = jnp.where(_lo_valid(), st[:16] if back == W else NEG, st[back:])
            m = functools.reduce(jnp.maximum, [c[8 * h:8 * h + 8] for c in ch.values() for h in range(2)])
            self.m[u] = jnp.max(m, axis=0, keepdims=True)
            for c, val in ch.items():
                self.s_ref(W * u + 16 * c, 16)[...] = val
            self.have[u] = sorted(ch)

    def probs(self, c, flush):
        lo, hi = [None] * 4, [None] * 4
        for u in range(4):
            if c not in self.have[u]:
                continue
            p = jnp.exp2(self.s_ref(W * u + 16 * c, 16)[...] - self.m[u])
            l = p[:8] + p[8:]
            self.l[u] = l if self.l[u] is None else self.l[u] + l
            if flush:
                self.s_ref(4 * W + 8 * u, 8)[...] = self.l[u]
            if c == u:
                hi[u] = jnp.where(_lo_valid(), 0.0, p)
                if self.a + 16 * u >= W:
                    lo[u] = jnp.where(_lo_valid(), p, 0.0)
            elif c < u:
                hi[u] = p
            else:
                lo[u] = p
        self.p[c - 16], self.p[c] = _butterfly(lo), _butterfly(hi)

    def out(self):
        k0 = max(0, self.a // 128 * 128 - W)
        k1 = self.a // 128 * 128 + 128
        ls = _butterfly([jnp.sum(l, axis=0, keepdims=True) for l in self.l])
        outs = [None] * 8
        for t in range(4):
            rows = [self.p.get(c, [None] * 4)[t] for c in range((k0 - self.a) // 16, (k1 - self.a) // 16)]
            p = jnp.concatenate([jnp.zeros((16, 128), f32) if r is None else r for r in rows], axis=0)
            o = jnp.dot(self.vload(t, k0, k1), p.astype(bf16), preferred_element_type=f32)
            o = o * pltpu.reciprocal(ls[t], full_range=False)
            outs[t], outs[4 + t] = o[:16], o[16:]
        y = jnp.concatenate(outs, axis=0).T
        z = [_sel(64, y[32 * p:32 * p + 16], y[32 * p + 16:32 * p + 32]) for p in range(4)]
        z = [_sel(16, z[p], z[p ^ 1]) for p in range(4)]
        z = [_sel(32, z[p], z[p ^ 2]) for p in range(4)]
        self.store(jnp.concatenate(z, axis=0))


def _interleave(*streams):
    keyed = []
    for k, stream in enumerate(streams):
        total = sum(c for c, _ in stream) or 1
        done = 0
        for j, (c, f) in enumerate(stream):
            keyed.append(((done + 0.5 * c) / total, k, j, f))
            done += c
    for _, _, _, f in sorted(keyed, key=lambda e: e[:3]):
        f()


def _kernel(x_hbm, wqkv_hbm, wo_hbm, wg_hbm, wu_hbm, wd_hbm, o_hbm,
            x_v, wqkv_v, wo_v, wg_v, wu_v, wd_v, q_v, k_v, vt_v, att_v, h_v, act_v, o_v, s_v, z_s, isem, osem,
            *, cfg):
    QR, QC, PR, PC, FR, FC, DR, DC, DK, LAG, WO, Q1, LS, TOK0, NBLK, WT = [
        cfg[k] for k in 'QR QC PR PC FR FC DR DC DK LAG WO Q1 LS TOK0 NBLK WT'.split()]
    srcs = {("x", i): (x_hbm.at[pl.ds(i * TM, TM)], x_v.at[pl.ds(i * TM, TM)]) for i in range(NB)}
    for j, name in enumerate("qkv"):
        srcs[name] = (wqkv_hbm.at[:, pl.ds(j * D, D)], wqkv_v.at[:, pl.ds(j * D, D)])
    srcs.update(o=(wo_hbm, wo_v), g=(wg_hbm, wg_v), u=(wu_hbm, wu_v), d=(wd_hbm, wd_v))
    copies = {k: pltpu.make_async_copy(s, d, isem.at[j]) for j, (k, (s, d)) in enumerate(srcs.items())}
    start = lambda *ks: (0, lambda: [copies[k].start() for k in ks])
    wait = lambda *ks: (0, lambda: [copies[k].wait() for k in ks])
    out_copies = []

    for k in (("x", 0), "k", "v", "q", ("x", 1)):
        copies[k].start()

    @pl.loop(0, 8)
    def _(j):
        z_s[j] = 0

    za, zb = z_s[0], z_s[1]
    pace = [True]

    def token(y):
        if pace[0]:
            s_v[pl.ds(pl.multiple_of(zb + 2 * SROWS, 8), 8), :] = y[:8, :128]

    def lhs(val, n):
        return [val[r0:r0 + n].astype(bf16) for r0 in range(0, TM, n)]

    def qkv_steps(i):
        st = {}

        def ln():
            st["xn"] = lhs(_ln(x_v[i * TM:i * TM + TM, :].astype(f32)), QR)

        def chunk(which, r0, c0):
            y = jnp.dot(st["xn"][r0 // QR], wqkv_v[:, which * D + c0:which * D + c0 + QC], preferred_element_type=f32)
            token(y)
            r = i * TM + r0
            if which == 0:
                q_v[r:r + QR, c0:c0 + QC] = (y * QSCALE).astype(bf16)
            elif which == 1:
                k_v[r:r + QR, c0:c0 + QC] = y.astype(bf16)
            else:
                for j in range(0, QR, 128):
                    vt_v[(r + j) // 128, c0:c0 + QC, :] = y[j:j + 128].T.astype(bf16)

        return [[(0, ln)]] + [[(QR * QC // 128, functools.partial(chunk, which, r0, c0))
                               for r0 in range(0, TM, QR) for c0 in range(0, D, QC)] for which in (1, 2, 0)]

    def unit(n):
        a, cols = 64 * (n // 4), slice(128 * (n % 4), 128 * (n % 4) + 128)

        def vload(t, k0, k1):
            return jnp.concatenate([jnp.concatenate(
                [vt_v[c, pl.ds(cols.start + 16 * hh, 16), :] for hh in (t, t + 4)], axis=0)
                for c in range(k0 // 128, k1 // 128)], axis=1)

        def store(val):
            att_v[a % (2 * TM):a % (2 * TM) + 64, cols] = val

        return _Attn(a, lambda u: pltpu.bitcast(q_v[a + 16 * u:a + 16 * u + 16, cols], i32),
                     lambda r, k: k_v[r:r + k, cols], vload, store,
                     lambda off, k: s_v.at[pl.ds(pl.multiple_of(za + (n % 2) * SROWS + off, 8), k), :])

    N = NBLK * TM // 16
    units = [unit(n) for n in range(N)]

    def attn_steps(n0, n1):
        steps = []
        for n in range(n0, n1):
            if n < N:
                steps += [(0, units[n].scores)]
            if 1 <= n <= N:
                steps += [(1, functools.partial(units[n - 1].probs, c, c % LS == LS - 1)) for c in range(16)]
            if LAG <= n < N + LAG:
                steps += [(WO, lambda: None), (0, units[n - LAG].out)]
        return steps

    def ffn_steps(i):
        st = {}

        def load_att():
            st["att"] = lhs(att_v[i % 2 * TM:i % 2 * TM + TM, :], PR)

        def proj(r0, c0):
            y = jnp.dot(st["att"][r0 // PR], wo_v[:, c0:c0 + PC], preferred_element_type=f32)
            token(y)
            h_v[r0:r0 + PR, c0:c0 + PC] = x_v[i * TM + r0:i * TM + r0 + PR, c0:c0 + PC].astype(f32) + y

        def ln():
            st["hn"] = lhs(_ln(h_v[...]), FR)

        def gate(r0, c0):
            st["g"] = jnp.dot(st["hn"][r0 // FR], wg_v[:, c0:c0 + FC], preferred_element_type=f32)
            token(st["g"])

        def up(r0, c0):
            u = jnp.dot(st["hn"][r0 // FR], wu_v[:, c0:c0 + FC], preferred_element_type=f32)
            token(u)
            hg = 0.5 * st.pop("g")
            act_v[r0:r0 + FR, c0:c0 + FC] = ((hg * jnp.tanh(hg) + hg) * u).astype(bf16)

        def down(r0, c0, k0):
            y = jnp.dot(act_v[r0:r0 + DR, k0:k0 + DK], wd_v[k0:k0 + DK, c0:c0 + DC], preferred_element_type=f32)
            token(y)
            st["acc"] = (h_v[r0:r0 + DR, c0:c0 + DC] if k0 == 0 else st["acc"]) + y
            if k0 + DK >= F:
                o_v[i * TM + r0:i * TM + r0 + DR, c0:c0 + DC] = st.pop("acc").astype(bf16)

        def flush(r0, n):
            r = pl.ds(i * TM + r0, n)
            out_copies.append(pltpu.make_async_copy(o_v.at[r], o_hbm.at[r], osem.at[len(out_copies)]))
            out_copies[-1].start()

        P = functools.partial
        head = [(0, load_att)] + [(PR * PC // 128, P(proj, r0, c0)) for r0 in range(0, TM, PR) for c0 in range(0, D, PC)]
        body = [(FR * FC // 128, P(f, r0, c0)) for r0 in range(0, TM, FR) for c0 in range(0, F, FC) for f in (gate, up)]
        tail = []
        for r0 in range(0, TM, DR):
            tail += [(DR * DC // 128 * min(DK, F - k0) // 512, P(down, r0, c0, k0))
                     for c0 in range(0, D, DC) for k0 in range(0, F, DK)]
            if i == NBLK - 1:
                tail += [(0, P(flush, r0, DR))]
        if i < NBLK - 1:
            tail += [(0, P(flush, 0, TM))]
        return head, [(0, ln)], body, tail

    ln0, k0, v0, q0 = qkv_steps(0)
    pace[0] = TOK0
    _interleave([wait(("x", 0))] + ln0 + [wait("k"), start("o", ("x", 2), "g")] + k0 + [wait("v"), start("u")] + v0
                + [wait("q"), start("d")] + q0 + [wait(("x", 1))])
    U = TM // 16
    _interleave(attn_steps(0, U), sum(qkv_steps(1), []))
    pace[0] = True
    for i in range(1, NBLK + 1):
        head, ln2, body, tail = ffn_steps(i - 1)
        if i == 1:
            head = [wait("o")] + head
            body = [wait("g", "u"), start(*[("x", j) for j in range(3, NB)])] + body
            tail = [wait("d")] + tail
        if i + 1 < NBLK:
            q = [wait(("x", i + 1))] + sum(qkv_steps(i + 1), [])
            dense = q[:2 + Q1] + head + ln2 + q[2 + Q1:] + body + tail
        else:
            dense = head + ln2 + body + tail
        if i < NBLK - 1:
            _interleave(attn_steps(i * U, i * U + U), dense)
        elif i == NBLK - 1:
            _interleave(attn_steps(i * U, i * U + LAG))
            _interleave(attn_steps(i * U + LAG, i * U + U + LAG) + [(WT, lambda: None)], dense)
        else:
            _interleave(dense)
    for j in range(NBLK, NB):
        if j >= 2:
            copies["x", j].wait()
    for c in out_copies:
        c.wait()


def make(flags=None, **kw):
    cfg = dict(QR=256, QC=128, PR=256, PC=128, FR=128, FC=128, DR=128, DC=256, DK=256, LAG=2, WO=4, Q1=8, LS=2, TOK0=False, NBLK=NB, WT=20)
    cfg.update(kw)

    @jax.jit
    def run(A_x, A_wqkv, A_wo, B_x, B_w_gate, B_w_up, B_w_down):
        anyspec = pl.BlockSpec(memory_space=pl.ANY)
        out = pl.pallas_call(
            functools.partial(_kernel, cfg=cfg),
            out_shape=jax.ShapeDtypeStruct((S, D), bf16),
            in_specs=[anyspec] * 6,
            out_specs=anyspec,
            scratch_shapes=[
                pltpu.VMEM((S, D), bf16), pltpu.VMEM((D, 3 * D), bf16), pltpu.VMEM((D, D), bf16),
                pltpu.VMEM((D, F), bf16), pltpu.VMEM((D, F), bf16), pltpu.VMEM((F, D), bf16),
                pltpu.VMEM((S, D), bf16), pltpu.VMEM((S, D), bf16), pltpu.VMEM((S // 128, D, 128), bf16),
                pltpu.VMEM((2 * TM, D), f32), pltpu.VMEM((TM, D), f32), pltpu.VMEM((TM, F), bf16),
                pltpu.VMEM((S, D), bf16), pltpu.VMEM((2 * SROWS + 8, 128), f32), pltpu.SMEM((8,), i32),
                pltpu.SemaphoreType.DMA((NB + 7,)), pltpu.SemaphoreType.DMA((NB + 4,)),
            ],
            compiler_params=pltpu.CompilerParams(vmem_limit_bytes=100 * 2 ** 20, flags=flags),
        )(A_x.reshape(S, D), A_wqkv, A_wo, B_w_gate, B_w_up, B_w_down)
        return out.reshape(1, S, D)
    return run


pallas_sequential_preLN__sliding_block__swiglu_ffn__prompt_kernel = make()
```

```python
import functools

import jax
import jax.numpy as jnp
import numpy as np
from jax import lax
from jax.experimental import pallas as pl
from jax.experimental.pallas import tpu as pltpu

S, D, DH, W, F = 2048, 512, 16, 256, 1792
EPS = 1e-5
QSCALE = float(DH ** -0.5 * np.log2(np.e))
NEG = -1e30
TM = 256
NB = S // TM
U = TM // 16
R = 64
SROWS = 4 * W + 32
PROWS = (W + 64) // 2
TOKEN, ZERO = 2 * SROWS, 2 * SROWS + 8
LAG = 2
OUT_POS, PRE_GAP, POST_GAP, DMA_GAP = 20, 1, 2, 6
FLUSH_EVERY, PULL_DELAY = 2, 1
PIECES = ((0, 1), (2, 3))
FAST_QKV, FAST_PROJ, FAST_FFN = 2, 1, 1
EARLY_SUMS = 5
TAIL_CUTS = (4, 9, 13)
FLAGS = {"XLA_TPU_EVENLY_DISTRIBUTE_CRITICAL_NODES": True}
NT = (((1,), (1,)), ((), ()))
f32, bf16, i32 = jnp.float32, jnp.bfloat16, jnp.int32
P = functools.partial


def _ln(x):
    m = jnp.mean(x, axis=-1, keepdims=True)
    c = x - m
    v = jnp.mean(c * c, axis=-1, keepdims=True)
    return c * lax.rsqrt(v + EPS)


def _sel(bit, x, y):
    ln = lax.broadcasted_iota(i32, x.shape, 1)
    return jnp.where((ln & bit) == 0, x, y)


def _lo_valid():
    return lax.broadcasted_iota(i32, (16, 128), 0) > (lax.broadcasted_iota(i32, (16, 128), 1) & 15)


def _butterfly(xs):
    for bit, d in ((32, 1), (64, 2)):
        ys = []
        for u in range(4):
            x, y = xs[u], xs[u ^ d]
            if x is None and y is None:
                ys.append(None)
            else:
                ys.append(_sel(bit, jnp.zeros_like(y) if x is None else x, jnp.zeros_like(x) if y is None else y))
        xs = ys
    return xs


class _Attn:
    def __init__(self, a, qload, kload, vload, store, s_ref, p_store, p_load):
        self.p_store, self.p_load = p_store, p_load
        self.a, self.qload, self.kload, self.vload, self.store, self.s_ref = a, qload, kload, vload, store, s_ref
        self.have, self.m, self.l = [None] * 4, [None] * 4, [None] * 4
        self.p = set()

    def scores(self):
        lane = lax.broadcasted_iota(i32, (8, 128), 1)
        for u in range(4):
            qu = self.qload(u)
            qbd = jnp.concatenate(
                [jnp.where((lane >> 4) == 4 * (s & 1) + ((s >> 1) ^ u), qu, 0) for s in range(8)], axis=0)
            back = min(W, self.a + 16 * u)
            st = lax.dot_general(self.kload(self.a + 16 * u - back, back + 16), pltpu.bitcast(qbd, bf16), NT,
                                 preferred_element_type=f32)
            nb = back // 16
            ch = {(u - nb + j) % 16: st[16 * j:16 * j + 16] for j in range(1 if back == W else 0, nb)}
            ch[u] = jnp.where(_lo_valid(), st[:16] if back == W else NEG, st[back:])
            m = functools.reduce(jnp.maximum, [c[8 * h:8 * h + 8] for c in ch.values() for h in range(2)])
            self.m[u] = jnp.max(m, axis=0, keepdims=True)
            for c, val in ch.items():
                self.s_ref(W * u + 16 * c, 16)[...] = val
            self.have[u] = sorted(ch)

    def probs(self, c, flush, us):
        for u in us:
            if c not in self.have[u]:
                continue
            p = jnp.exp2(self.s_ref(W * u + 16 * c, 16)[...] - self.m[u])
            l = p[:8] + p[8:]
            self.l[u] = l if self.l[u] is None else self.l[u] + l
            if flush:
                self.s_ref(4 * W + 8 * u, 8)[...] = self.l[u]
            if c == u:
                parts = {c: jnp.where(_lo_valid(), 0.0, p)}
                if self.a + 16 * u >= W:
                    parts[c - 16] = jnp.where(_lo_valid(), p, 0.0)
            else:
                parts = {c if c < u else c - 16: p}
            for kc, val in parts.items():
                self.p_store(u, kc + 16, val.astype(bf16))
                self.p.add((u, kc))

    def out(self):
        k0 = max(0, self.a // 128 * 128 - W)
        k1 = self.a // 128 * 128 + 128
        ls = _butterfly([jnp.sum(l, axis=0, keepdims=True) for l in self.l])
        words = [_butterfly([self.p_load(u, kc + 16) if (u, kc) in self.p else None for u in range(4)])
                 for kc in range((k0 - self.a) // 16, (k1 - self.a) // 16)]
        outs = [None] * 8
        for t in range(4):
            p = jnp.concatenate([jnp.zeros((8, 128), i32) if w[t] is None else w[t] for w in words], axis=0)
            p = pltpu.bitcast(p, bf16)
            o = jnp.dot(self.vload(t, k0, k1), p, preferred_element_type=f32)
            o = o * pltpu.reciprocal(ls[t], full_range=False)
            outs[t], outs[4 + t] = o[:16], o[16:]
        y = jnp.concatenate(outs, axis=0).T
        z = [_sel(64, y[32 * p:32 * p + 16], y[32 * p + 16:32 * p + 32]) for p in range(4)]
        z = [_sel(16, z[p], z[p ^ 1]) for p in range(4)]
        z = [_sel(32, z[p], z[p ^ 2]) for p in range(4)]
        self.store(jnp.concatenate(z, axis=0))


def _interleave(*streams):
    keyed = []
    for k, stream in enumerate(streams):
        total = sum(c for c, _ in stream) or 1
        done = 0
        for j, (c, f) in enumerate(stream):
            keyed.append(((done + 0.5 * c) / total, k, j, f))
            done += c
    for _, _, _, f in sorted(keyed, key=lambda e: e[:3]):
        f()


def _kernel(x_hbm, wqkv_hbm, wo_hbm, wg_hbm, wu_hbm, wd_hbm, o_hbm,
            x_v, wqkv_v, wo_v, wg_v, wu_v, wd_v, q_v, k_v, vt_v, att_v, h_v, act_v, o_v, s_v, z_s,
            p_v, acts_v, wq_s, wk_s, wv_s, wo_s, wg_s, wu_s, wd_s, isem, osem):
    q_v, k_v, vt_v, act_v, acts_v, wq_s, wk_s, wv_s, wo_s, wg_s, wu_s, wd_s = [
        r.bitcast(bf16) for r in (q_v, k_v, vt_v, act_v, acts_v, wq_s, wk_s, wv_s, wo_s, wg_s, wu_s, wd_s)]
    p_v = p_v.bitcast(bf16)
    srcs = {name: (x_hbm.at[pl.ds(r0, r1 - r0)], x_v.at[pl.ds(r0, r1 - r0)])
            for name, r0, r1 in (("x0", 0, TM), ("x1", TM, 3 * TM), ("x2", 3 * TM, S))}
    for j, name in enumerate("qkv"):
        srcs[name] = (wqkv_hbm.at[:, pl.ds(j * D, D)], wqkv_v.at[:, pl.ds(j * D, D)])
    srcs.update(o=(wo_hbm, wo_v), g=(wg_hbm, wg_v), u=(wu_hbm, wu_v), d=(wd_hbm, wd_v))
    copies = {k: pltpu.make_async_copy(s, d, isem.at[j]) for j, (k, (s, d)) in enumerate(srcs.items())}
    start = lambda *ks: (0, lambda: [copies[k].start() for k in ks])
    done = set()
    wait = lambda *ks: (0, lambda: [(copies[k].wait(), done.add(k)) for k in ks])
    out_copies = []
    wrefs = dict(q=(wqkv_v, 0, D, D, wq_s), k=(wqkv_v, D, D, D, wk_s), v=(wqkv_v, 2 * D, D, D, wv_s),
                 o=(wo_v, 0, D, D, wo_s), g=(wg_v, 0, D, F, wg_s), u=(wu_v, 0, D, F, wu_s), d=(wd_v, 0, F, D, wd_s))

    copies["x0"].start()
    copies["k"].start()

    @pl.loop(0, 8)
    def _(j):
        z_s[j] = 0

    za, zb = z_s[0], z_s[1]
    s_rows = lambda base, r, n: s_v.at[pl.ds(pl.multiple_of(base + r, 8), n), :]
    s_v[ZERO:ZERO + 8, :] = jnp.zeros((8, 128), f32)
    due = []

    def token(y):
        due[:] = [d - 1 for d in due]
        if due and due[0] <= 0:
            due[:] = [d for d in due if d > 0]
            top = y[:8, :128] + s_rows(zb, ZERO, 8)[...]
            if y.shape[1] > 128:
                top = jnp.concatenate([top, y[:8, 128:]], axis=1)
            y = jnp.concatenate([top, y[8:]], axis=0)
        s_rows(zb, TOKEN, 8)[...] = y[8:16, :128]
        return y

    def prep(name):
        w, c_base, K, Nn, sums = wrefs[name]

        def run(r0, c0):
            assert name in done
            cw = min(256, Nn // 2 - c0)
            b11, b12, b21, b22 = [w[r:r + 16, c_base + c:c_base + c + cw].astype(f32)
                                  for r in (r0, K // 2 + r0) for c in (c0, Nn // 2 + c0)]
            zero = s_rows(za, ZERO, 8)[...]
            zero = jnp.concatenate([jnp.concatenate([zero] * (cw // 128), axis=1)] * (16 // 8), axis=0)
            b11, b22 = b11 + zero, b22 + zero
            for j, v in enumerate((b11 + b22, b12 - b22, b21 - b11, b11 + b12, b21 + b22)):
                sums[pl.ds(j * K // 2 + r0, 16), c0:c0 + cw] = v.astype(bf16)
            done.add(("sum", name, r0, c0))
        return [(1, P(run, r0, c0)) for c0 in range(0, Nn // 2, 256) for r0 in range(0, K // 2, 16)]

    def left(a11, a12, a21, a22):
        return [v.astype(bf16) for v in (a11 + a22, a21 + a22, a11, a22, a11 + a12, a21 - a11, a12 - a22)]

    def left_of(val):
        return left(*[val[r:r + R, c:c + D // 2] for r in (0, R) for c in (0, D // 2)])

    def strassen(name, lget, c0, cw, emit):
        w, c_base, K, Nn, sums = wrefs[name]
        st = {}

        def prod(i):
            assert all(("sum", name, r, c0 // 256 * 256) in done for r in range(0, K // 2, 16))
            if i == 2:
                rhs = w[:K // 2, c_base + c0:c_base + c0 + cw]
            elif i == 5:
                rhs = w[K // 2:, c_base + Nn // 2 + c0:c_base + Nn // 2 + c0 + cw]
            else:
                rhs = sums[pl.ds((1, 3, 4, 6, 7).index(i) * K // 2, K // 2), c0:c0 + cw]
            m = jnp.dot(lget(i - 1), rhs, preferred_element_type=f32)
            m = token(m)
            if i == 2:
                st[2] = m
            elif i == 4:
                emit(1, 0, st[2] + m)
                st[4] = m
            elif i == 5:
                st[11], st[5] = st.pop(4) - m, m
            elif i == 3:
                emit(0, 1, m + st.pop(5))
                st[22] = m - st.pop(2)
            elif i == 1:
                st[11], st[22] = st[11] + m, st[22] + m
            elif i == 7:
                emit(0, 0, st.pop(11) + m)
            else:
                emit(1, 1, st.pop(22) + m)
        return [(R * cw // 128 * K // 1024, P(prod, i)) for i in (2, 4, 5, 3, 1, 7, 6)]

    def qkv_steps(i):
        st = {}

        fast = i >= FAST_QKV

        def ln(r0):
            assert ("x0", "x1", "x1", "x2")[min(i, 3)] in done
            x = x_v[i * TM + r0:i * TM + r0 + 2 * R, :].astype(f32)
            xn = _ln(x)
            st["xn", r0] = left_of(xn) if fast else xn.astype(bf16)

        def put(name, r0, c0, y):
            r, n, cols = i * TM + r0, y.shape[0], slice(c0, c0 + y.shape[1])
            if name == "q":
                q_v[r:r + n, cols] = (y * QSCALE).astype(bf16)
            elif name == "k":
                k_v[r:r + n, cols] = y.astype(bf16)
            elif n < 128:
                st[r, c0] = y
                if (r ^ n, c0) in st:
                    put(name, r0 & ~n, c0, jnp.concatenate([st.pop((r & ~n, c0)), st.pop((r | n, c0))], axis=0))
            else:
                for j in range(0, n, 128):
                    done.add(("v", r + j, c0))
                    vt_v[cols, r + j:r + j + 128] = y[j:j + 128].T.astype(bf16)

        def chunk(name, r0, c0):
            c = wrefs[name][1] + c0
            y = jnp.dot(st["xn", r0], wqkv_v[:, c:c + 128], preferred_element_type=f32)
            y = token(y)
            put(name, r0, c0, y)

        lns = [(0, P(ln, r0)) for r0 in range(0, TM, 2 * R)]
        if fast:
            return [lns] + [[s for r0 in range(0, TM, 2 * R) for c0 in range(0, D // 2, 128) for s in strassen(
                name, lambda j, r0=r0: st["xn", r0][j], c0, 128,
                lambda a, b, y, name=name, r0=r0, c0=c0: put(name, r0 + a * R, c0 + b * D // 2, y))] for name in "kvq"]
        return [lns] + [[(128 * 128 // 128, P(chunk, name, r0, c0))
                               for r0 in range(0, TM, 128) for c0 in range(0, D, 128)] for name in "kvq"]

    def unit(n):
        a, cols = 64 * (n // 4), slice(128 * (n % 4), 128 * (n % 4) + 128)

        def vload(t, k0, k1):
            assert all(("v", r, cols.start) in done for r in range(k0, k1, 128))
            return jnp.concatenate([vt_v[pl.ds(cols.start + 16 * hh, 16), k0:k1] for hh in (t, t + 4)], axis=0)

        def store(val):
            done.add(n)
            att_v[a % (2 * TM):a % (2 * TM) + 64, cols] = val

        p_at = lambda u, c: (pl.ds(n % (LAG + 1) * 2 * PROWS + 16 * c, 16), pl.ds(128 * u, 128))

        def p_store(u, c, val):
            p_v[p_at(u, c)] = val

        return _Attn(a, lambda u: pltpu.bitcast(q_v[a + 16 * u:a + 16 * u + 16, cols], i32),
                     lambda r, k: k_v[r:r + k, cols], vload, store,
                     lambda off, k: s_rows(za, n % 2 * SROWS + off, k), p_store,
                     lambda u, c: pltpu.bitcast(p_v[p_at(u, c)], i32))

    N = NB * U
    units = [unit(n) for n in range(N)]

    def probs(n, c, us):
        flush = c % FLUSH_EVERY == FLUSH_EVERY - 1
        units[n].probs(c, flush, us)
        if flush:
            due.append(PULL_DELAY)

    def attn_steps(n0, n1):
        steps = []
        for n in range(n0, n1):
            steps += sites.get(n, [])
            if n < N:
                steps += [(0, units[n].scores)]
            ps = []
            if 1 <= n <= N:
                ps = [(len(us) / 4, P(probs, n - 1, c, us)) for c in range(16) for us in PIECES]
            if LAG <= n < N + LAG:
                ps.insert(min(OUT_POS, len(ps)), (0, units[n - LAG].out))
            steps += [(PRE_GAP, lambda: None)] + ps + [(POST_GAP, lambda: None)]
        return steps

    def ffn_steps(i):
        st = {}

        def load_att(r0):
            assert done >= {"o", "g", "u"} and done >= set(range(i * U + r0 // 16, i * U + (r0 + 2 * R) // 16))
            att = att_v[i % 2 * TM + r0:i % 2 * TM + r0 + 2 * R, :]
            st["att", r0] = left_of(att) if i >= FAST_PROJ else att.astype(bf16)

        def put_h(r0, c0, y):
            n, cols = y.shape[0], slice(c0, c0 + y.shape[1])
            h_v[i % 2, r0:r0 + n, cols] = x_v[i * TM + r0:i * TM + r0 + n, cols].astype(f32) + y

        def proj(r0, c0):
            y = jnp.dot(st["att", r0], wo_v[:, c0:c0 + 128], preferred_element_type=f32)
            y = token(y)
            put_h(r0, c0, y)

        def ln(r0):
            hn = _ln(h_v[i % 2, r0:r0 + 2 * R, :])
            if i >= FAST_FFN:
                st["hn", r0] = left_of(hn)
            else:
                st["hn", r0], st["hn", r0 + R] = hn[:R].astype(bf16), hn[R:].astype(bf16)

        def swiglu(g, u):
            hg = 0.5 * g
            return (hg * jnp.tanh(hg) + hg) * u

        def gate(r0, c0):
            st["g"] = jnp.dot(st["hn", r0], wg_v[:, c0:c0 + 128], preferred_element_type=f32)
            st["g"] = token(st["g"])

        def up(r0, c0):
            u = jnp.dot(st["hn", r0], wu_v[:, c0:c0 + 128], preferred_element_type=f32)
            u = token(u)
            act_v[r0:r0 + 64, c0:c0 + 128] = swiglu(st.pop("g"), u).astype(bf16)

        def put_g(a, b, y):
            st["g", a, b] = y

        def put_u(r0, c0, a, b, y):
            st["a", a, b] = swiglu(st.pop(("g", a, b)), y)
            if (a, b) == (1, 1):
                ops = left(*[st.pop(("a", p, q)) for p in (0, 1) for q in (0, 1)])
                for j, v in enumerate(ops):
                    acts_v[pl.ds((j * TM + r0) // 2, R), c0:c0 + 128] = v

        def put_o(r0, c0, y):
            n, cols = y.shape[0], slice(c0, c0 + y.shape[1])
            o_v[i * TM + r0:i * TM + r0 + n, cols] = (h_v[i % 2, r0:r0 + n, cols] + y).astype(bf16)

        def down(r0, c0, k0):
            assert "d" in done
            y = jnp.dot(act_v[r0:r0 + 64, k0:k0 + 256], wd_v[k0:k0 + 256, c0:c0 + 256], preferred_element_type=f32)
            y = token(y)
            st["acc"] = y if k0 == 0 else st["acc"] + y
            if k0 + 256 >= F:
                put_o(r0, c0, st.pop("acc"))

        if i >= FAST_PROJ:
            head = [s for r0 in range(0, TM, 2 * R) for c0 in range(0, D // 2, 128) for s in strassen(
                "o", lambda j, r0=r0: st["att", r0][j], c0, 128,
                lambda a, b, y, r0=r0, c0=c0: put_h(r0 + a * R, c0 + b * D // 2, y))]
        else:
            head = [(128 * 128 // 128, P(proj, r0, c0)) for r0 in range(0, TM, 128) for c0 in range(0, D, 128)]
        if i >= FAST_FFN:
            body, tail = [], []
            for r0 in range(0, TM, 2 * R):
                hget = lambda j, r0=r0: st["hn", r0][j]
                for c0 in range(0, F // 2, 128):
                    body += strassen("g", hget, c0, 128, put_g) + strassen("u", hget, c0, 128, P(put_u, r0, c0))
                for c0 in range(0, D // 2, 128):
                    tail += strassen("d", lambda j, r0=r0: acts_v[pl.ds((j * TM + r0) // 2, R), :], c0, 128,
                                     lambda a, b, y, r0=r0, c0=c0: put_o(r0 + a * R, c0 + b * D // 2, y))
        else:
            body = [(64 * 128 // 128, P(f, r0, c0)) for r0 in range(0, TM, 64) for c0 in range(0, F, 128) for f in (gate, up)]
            tail = [(64 * 256 // 128 * min(256, F - k0) // 512, P(down, r0, c0, k0))
                    for r0 in range(0, TM, 64) for c0 in range(0, D, 256) for k0 in range(0, F, 256)]
        n = len(head) // 2
        heads = [[(0, P(load_att, r0))] + part + [(0, P(ln, r0))] for r0, part in ((0, head[:n]), (2 * R, head[n:]))]
        return heads, body, tail

    def flush(r0, r1):
        def run():
            r = pl.ds(r0, r1 - r0)
            out_copies.append(pltpu.make_async_copy(o_v.at[r], o_hbm.at[r], osem.at[len(out_copies)]))
            out_copies[-1].start()
        return (0, run)

    def spread(steps, extra):
        out = list(steps)
        for j, (_, f) in reversed(list(enumerate(extra))):
            out.insert(j * len(steps) // len(extra), (0, f))
        return out

    gap = (DMA_GAP, lambda: None)
    sites = {3: [gap, wait("x1")], U + 3: [gap, wait("o", "g", "u"), start("d", "x2")], 2 * U: [wait("d", "x2")]}
    ln0, k0, v0, q0 = qkv_steps(0)
    ln1, k1, v1, q1 = qkv_steps(1)
    nxt = qkv_steps(2)
    _interleave([wait("x0"), start("q")] + ln0 + [wait("k"), start("v")] + k0
                + [wait("q"), start("x1")] + q0 + [wait("v"), start("o", "g", "u")])
    _interleave(attn_steps(0, U), v0 + ln1 + spread(k1 + nxt[0][:1] + v1 + nxt[0][1:] + q1, prep("k") + prep("v")))
    gu = [s for pair in zip(prep("g"), prep("u")) for s in pair]
    cut = len(gu) * EARLY_SUMS // 8
    prev_tail = []
    for i in range(1, NB + 1):
        (head_a, head_b), body, tail = ffn_steps(i - 1)
        lnx, kk, vv, qq = nxt if i == 1 else qkv_steps(i + 1) if i + 1 < NB else ([], [], [], [])
        t1, t2, t3 = [len(prev_tail) * n // 14 for n in TAIL_CUTS]
        if i == 1:
            dense = (spread(kk + vv, prep("q")) + qq[:14] + spread(
                head_a + qq[14:21] + head_b + qq[21:], prep("o")) + spread(body, gu[:cut]))
        else:
            first = lnx[:1] + prev_tail[:t1] + head_a + prev_tail[t1:t2]
            mid = first + head_b + prev_tail[t2:t3] + lnx[1:] + prev_tail[t3:] + kk + vv + qq
            if i == 2:
                mid, body = spread(mid, gu[cut:]), spread(body, prep("d"))
            dense = mid + body
        if i < NB:
            _interleave(attn_steps(i * U, i * U + U), dense)
        else:
            _interleave(attn_steps(N, N + LAG) + [(10, lambda: None)], first)
            half = len(tail) // 2
            _interleave(dense[len(first):] + [flush(0, S - TM)] + tail[:half] + [flush(S - TM, S - TM // 2)] + tail[half:]
                        + [flush(S - TM // 2, S)])
        prev_tail = tail
    for c in out_copies:
        c.wait()


@jax.jit
def pallas_sequential_preLN__sliding_block__swiglu_ffn__prompt_kernel(
    A_x: jax.Array,
    A_wqkv: jax.Array,
    A_wo: jax.Array,
    B_x: jax.Array,
    B_w_gate: jax.Array,
    B_w_up: jax.Array,
    B_w_down: jax.Array,
):
    del B_x
    hbm = pl.BlockSpec(memory_space=pl.ANY)
    vmem = pltpu.VMEM
    out = pl.pallas_call(
        _kernel,
        out_shape=jax.ShapeDtypeStruct((S, D), bf16),
        in_specs=[hbm] * 6,
        out_specs=hbm,
        scratch_shapes=[
            vmem((S, D), bf16), vmem((D, 3 * D), bf16), vmem((D, D), bf16),
            vmem((D, F), bf16), vmem((D, F), bf16), vmem((F, D), bf16),
            vmem((S // 2, D), i32), vmem((S // 2, D), i32), vmem((D // 2, S), i32),
            vmem((2 * TM, D), f32), vmem((2, TM, D), f32), vmem((TM // 2, F), i32),
            vmem((S, D), bf16), vmem((2 * SROWS + 16, 128), f32), pltpu.SMEM((8,), i32),
            vmem(((LAG + 1) * PROWS, 512), i32),
            vmem((7 * TM // 4, F // 2), i32),
            *[vmem((5 * D // 4, D // 2), i32)] * 4, *[vmem((5 * D // 4, F // 2), i32)] * 2,
            vmem((5 * F // 4, D // 2), i32),
            pltpu.SemaphoreType.DMA((10,)), pltpu.SemaphoreType.DMA((3,)),
        ],
        compiler_params=pltpu.CompilerParams(vmem_limit_bytes=100 * 2 ** 20, flags=FLAGS),
    )(A_x.reshape(S, D), A_wqkv, A_wo, B_w_gate, B_w_up, B_w_down)
    return out.reshape(1, S, D)
```
